```python
import os as _os
_os.environ.setdefault('JAX_PLATFORMS', 'cpu')
import jax
import jax.numpy as jnp

def _softmax(x, axis=-1):
    return jax.nn.softmax(x, axis=axis)

def _gelu(x):
    return jax.nn.gelu(x, approximate=True)

def _silu(x):
    return jax.nn.silu(x)

def _sigmoid(x):
    return jax.nn.sigmoid(x)

def _layernorm(x, axis=-1, eps=1e-05):
    m = jnp.mean(x, axis=axis, keepdims=True)
    v = jnp.var(x, axis=axis, keepdims=True)
    return (x - m) / jnp.sqrt(v + eps)

def _scatter_add(tgt, idx, src, axis=0):
    return tgt.at[idx].add(src)

def _segment_sum(src, seg, n):
    return jax.ops.segment_sum(src, seg, n)

class _Rng:

    def __init__(self, key):
        self._k = key

    def _next(self):
        self._k, sub = jax.random.split(self._k)
        return sub

    def normal(self, shape):
        return jax.random.normal(self._next(), shape, dtype=jnp.bfloat16)

    def randint(self, lo, hi, shape):
        return jax.random.randint(self._next(), shape, lo, hi, dtype=jnp.int32)

    def uniform(self, shape, lo=0.0, hi=1.0):
        return jax.random.uniform(self._next(), shape, jnp.bfloat16, lo, hi)

    def permutation(self, n):
        return jax.random.permutation(self._next(), n)
kernel_name = 'standalone__autoregressive_conv_wavenet__speech'

def setup_inputs():
    _rng = _Rng(jax.random.key(int.from_bytes(__import__("os").urandom(4), "little")))
    _w = lambda a: (lambda t: t.astype(jnp.bfloat16) if jnp.issubdtype(t.dtype, jnp.floating) else t)(jnp.asarray(a))
    B, T, D, K = (2, 4000, 512, 31)
    return {'x': _w((lambda *s: _rng.normal(s) * 0.05)(B, T, D)), 'w': _w((lambda *s: _rng.normal(s) * 0.05)(K, D, 2 * D)), 'w_o': _w((lambda *s: _rng.normal(s) * 0.05)(D, D))}

def reference(x, w, w_o):
    B, T, D = x.shape
    K = w.shape[0]
    dil = 2
    pad = (K - 1) * dil
    xp = jnp.pad(x, ((0, 0), (pad, 0), (0, 0)))
    h = jnp.einsum('btc,cd->btd', xp[:, pad:pad + T, :], w[0])
    for i in range(1, K):
        off = pad - i * dil
        h = h + jnp.einsum('btc,cd->btd', xp[:, off:off + T, :], w[i])
    f = h[..., :D].copy()
    g = h[..., D:].copy()
    z = jnp.tanh(f) * _sigmoid(g)
    return z @ w_o
```

```python
import jax
import jax.numpy as jnp
import jax.experimental.pallas as pl
import jax.experimental.pallas.tpu as pltpu

_HALO = 64


@jax.jit
def pallas_standalone__autoregressive_conv_wavenet__speech_kernel(
    x: jax.Array,
    w: jax.Array,
    w_o: jax.Array,
):
    B, T, D = x.shape
    K = w.shape[0]
    N = w.shape[2]
    dil = 2
    H = _HALO
    assert (K - 1) * dil <= H
    tm = 4000
    assert T % tm == 0 and tm >= H
    nt = T // tm

    def kernel(x_ref, w_hbm, wo_ref, o_ref, xs, acc, wv, sems):
        b = pl.program_id(0)
        j = pl.program_id(1)
        first = jnp.logical_and(b == 0, j == 0)

        @pl.when(first)
        def _():
            for i in range(K):
                pltpu.make_async_copy(w_hbm.at[i], wv.at[i], sems.at[i]).start()

        @pl.when(j == 0)
        def _():
            xs[0:H, :] = jnp.zeros((H, D), x_ref.dtype)

        @pl.when(j > 0)
        def _():
            xs[0:H, :] = xs[tm:tm + H, :]

        xs[H:H + tm, :] = x_ref[0]

        for i in range(K):
            @pl.when(first)
            def _():
                pltpu.make_async_copy(w_hbm.at[i], wv.at[i], sems.at[i]).wait()

            lhs = xs[H - dil * i:H - dil * i + tm, :]
            p = jnp.dot(lhs, wv[i], preferred_element_type=jnp.float32)
            if i == 0:
                acc[...] = p
            else:
                acc[...] += p

        h = acc[...]
        z = jnp.tanh(h[:, :D]) * jax.nn.sigmoid(h[:, D:])
        o_ref[0] = jnp.dot(
            z.astype(jnp.bfloat16), wo_ref[...], preferred_element_type=jnp.float32
        ).astype(o_ref.dtype)

    return pl.pallas_call(
        kernel,
        grid=(B, nt),
        in_specs=[
            pl.BlockSpec((1, tm, D), lambda b, j: (b, j, 0)),
            pl.BlockSpec(memory_space=pl.ANY),
            pl.BlockSpec((D, D), lambda b, j: (0, 0)),
        ],
        out_specs=pl.BlockSpec((1, tm, D), lambda b, j: (b, j, 0)),
        out_shape=jax.ShapeDtypeStruct((B, T, D), x.dtype),
        scratch_shapes=[
            pltpu.VMEM((tm + H, D), x.dtype),
            pltpu.VMEM((tm, N), jnp.float32),
            pltpu.VMEM((K, D, N), w.dtype),
            pltpu.SemaphoreType.DMA((K,)),
        ],
        compiler_params=pltpu.CompilerParams(
            dimension_semantics=("arbitrary", "arbitrary"),
            vmem_limit_bytes=100 * 1024 * 1024,
        ),
    )(x, w, w_o)
```

```python
import jax
import jax.numpy as jnp
import jax.experimental.pallas as pl
import jax.experimental.pallas.tpu as pltpu

_HALO = 64
_TILE = 2000


@jax.jit
def pallas_standalone__autoregressive_conv_wavenet__speech_kernel(
    x: jax.Array,
    w: jax.Array,
    w_o: jax.Array,
):
    B, T, D = x.shape
    K = w.shape[0]
    N = w.shape[2]
    dil = 2
    H = _HALO
    tm = _TILE
    assert dil == 2 and (K - 1) * dil <= H - 2 and H % 8 == 0
    assert T % tm == 0 and tm >= H and tm % 8 == 0
    nt = T // tm
    R = tm + H

    def kernel(x_ref, w_hbm, wo_ref, o_ref, xs, acc, wv, sems):
        b = pl.program_id(0)
        j = pl.program_id(1)
        first = jnp.logical_and(b == 0, j == 0)

        @pl.when(first)
        def _():
            for i in range(K):
                pltpu.make_async_copy(w_hbm.at[i], wv.at[i], sems.at[i]).start()

        @pl.when(j == 0)
        def _():
            xs[0, 0:H, :] = jnp.zeros((H, D), x_ref.dtype)

        @pl.when(j > 0)
        def _():
            xs[0, 0:H, :] = xs[0, tm:tm + H, :]

        xs[0, H:H + tm, :] = x_ref[0]

        for r in range(1, 4):
            xs[r, 8:R, :] = xs[0, 8 - dil * r:R - dil * r, :]

        def wait_w(i):
            @pl.when(first)
            def _():
                pltpu.make_async_copy(w_hbm.at[i], wv.at[i], sems.at[i]).wait()

        wait_w(0)
        acc[...] = jnp.dot(xs[0, H:H + tm, :], wv[0],
                           preferred_element_type=jnp.float32)

        def body(i, carry):
            wait_w(i)
            r = jnp.bitwise_and(i, 3)
            a = jnp.right_shift(i, 2)
            start = pl.multiple_of(H - 8 * a, 8)
            lhs = xs[r, pl.ds(start, tm), :]
            acc[...] += jnp.dot(lhs, wv[i], preferred_element_type=jnp.float32)
            return carry

        jax.lax.fori_loop(1, K, body, 0)

        h = acc[...]
        z = jnp.tanh(h[:, :D]) * jax.nn.sigmoid(h[:, D:])
        o_ref[0] = jnp.dot(
            z.astype(jnp.bfloat16), wo_ref[...], preferred_element_type=jnp.float32
        ).astype(o_ref.dtype)

    return pl.pallas_call(
        kernel,
        grid=(B, nt),
        in_specs=[
            pl.BlockSpec((1, tm, D), lambda b, j: (b, j, 0)),
            pl.BlockSpec(memory_space=pl.ANY),
            pl.BlockSpec((D, D), lambda b, j: (0, 0)),
        ],
        out_specs=pl.BlockSpec((1, tm, D), lambda b, j: (b, j, 0)),
        out_shape=jax.ShapeDtypeStruct((B, T, D), x.dtype),
        scratch_shapes=[
            pltpu.VMEM((4, R, D), x.dtype),
            pltpu.VMEM((tm, N), jnp.float32),
            pltpu.VMEM((K, D, N), w.dtype),
            pltpu.SemaphoreType.DMA((K,)),
        ],
        compiler_params=pltpu.CompilerParams(
            dimension_semantics=("arbitrary", "arbitrary"),
            vmem_limit_bytes=110 * 1024 * 1024,
        ),
    )(x, w, w_o)
```

```python
import jax
import jax.numpy as jnp
import jax.experimental.pallas as pl
import jax.experimental.pallas.tpu as pltpu

_HALO = 64
_TILE = 2000


@jax.jit
def pallas_standalone__autoregressive_conv_wavenet__speech_kernel(
    x: jax.Array,
    w: jax.Array,
    w_o: jax.Array,
):
    B, T, D = x.shape
    K = w.shape[0]
    N = w.shape[2]
    dil = 2
    H = _HALO
    tm = _TILE
    assert dil == 2 and K % 2 == 1 and (K - 1) * dil <= H - 4 and H % 8 == 0
    assert T % tm == 0 and tm >= H and tm % 8 == 0
    nt = T // tm
    R = tm + H
    n_pairs = (K - 1) // 2

    def kernel(x_ref, w_hbm, wo_ref, o_ref, xb, xw, acc, wv, sems):
        b = pl.program_id(0)
        j = pl.program_id(1)
        first = jnp.logical_and(b == 0, j == 0)

        def w_copy(i):
            return pltpu.make_async_copy(
                w_hbm.at[i], wv.at[pl.ds(i * D, D), :], sems.at[i])

        @pl.when(first)
        def _():
            for i in range(K):
                w_copy(i).start()

        @pl.when(j == 0)
        def _():
            xb[0:H, :] = jnp.zeros((H, D), x_ref.dtype)

        @pl.when(j > 0)
        def _():
            xb[0:H, :] = xb[tm:tm + H, :]

        xb[H:H + tm, :] = x_ref[0]

        for s in range(2):
            lo = 8 - dil * (2 * s + 1)
            xw[s, 8:R, 0:D] = xb[lo:lo + R - 8, :]
            lo = 8 - dil * (2 * s + 2)
            xw[s, 8:R, D:2 * D] = xb[lo:lo + R - 8, :]

        def wait_w(i):
            @pl.when(first)
            def _():
                w_copy(i).wait()

        wait_w(0)
        acc[...] = jnp.dot(xb[H:H + tm, :], wv[0:D, :],
                           preferred_element_type=jnp.float32)

        def body(p, carry):
            wait_w(2 * p + 1)
            wait_w(2 * p + 2)
            s = jnp.bitwise_and(p, 1)
            a = jnp.right_shift(p, 1)
            start = pl.multiple_of(H - 8 * a, 8)
            lhs = xw[s, pl.ds(start, tm), :]
            w_start = pl.multiple_of((2 * p + 1) * D, D)
            rhs = wv[pl.ds(w_start, 2 * D), :]
            acc[...] += jnp.dot(lhs, rhs, preferred_element_type=jnp.float32)
            return carry

        jax.lax.fori_loop(0, n_pairs, body, 0)

        h = acc[...]
        z = jnp.tanh(h[:, :D]) * (0.5 + 0.5 * jnp.tanh(0.5 * h[:, D:]))
        o_ref[0] = jnp.dot(
            z.astype(jnp.bfloat16), wo_ref[...], preferred_element_type=jnp.float32
        ).astype(o_ref.dtype)

    return pl.pallas_call(
        kernel,
        grid=(B, nt),
        in_specs=[
            pl.BlockSpec((1, tm, D), lambda b, j: (b, j, 0)),
            pl.BlockSpec(memory_space=pl.ANY),
            pl.BlockSpec((D, D), lambda b, j: (0, 0)),
        ],
        out_specs=pl.BlockSpec((1, tm, D), lambda b, j: (b, j, 0)),
        out_shape=jax.ShapeDtypeStruct((B, T, D), x.dtype),
        scratch_shapes=[
            pltpu.VMEM((R, D), x.dtype),
            pltpu.VMEM((2, R, 2 * D), x.dtype),
            pltpu.VMEM((tm, N), jnp.float32),
            pltpu.VMEM((K * D, N), w.dtype),
            pltpu.SemaphoreType.DMA((K,)),
        ],
        compiler_params=pltpu.CompilerParams(
            dimension_semantics=("arbitrary", "arbitrary"),
            vmem_limit_bytes=110 * 1024 * 1024,
        ),
    )(x, w, w_o)
```
